```python
import os as _os
_os.environ.setdefault("JAX_PLATFORMS", "cpu")
import jax
import jax.numpy as jnp

def _softmax(x, axis=-1):
    return jax.nn.softmax(x, axis=axis)
def _gelu(x):
    return jax.nn.gelu(x, approximate=True)
def _silu(x):
    return jax.nn.silu(x)
def _sigmoid(x):
    return jax.nn.sigmoid(x)
def _layernorm(x, axis=-1, eps=1e-5):
    m = jnp.mean(x, axis=axis, keepdims=True)
    v = jnp.var(x, axis=axis, keepdims=True)
    return (x - m) / jnp.sqrt(v + eps)
def _scatter_add(tgt, idx, src, axis=0):
    return tgt.at[idx].add(src)
def _segment_sum(src, seg, n):
    return jax.ops.segment_sum(src, seg, n)
class _Rng:
    def __init__(self, key):
        self._k = key
    def _next(self):
        self._k, sub = jax.random.split(self._k)
        return sub
    def normal(self, shape):
        return jax.random.normal(self._next(), shape, dtype=jnp.bfloat16)
    def randint(self, lo, hi, shape):
        return jax.random.randint(self._next(), shape, lo, hi, dtype=jnp.int32)
    def uniform(self, shape, lo=0.0, hi=1.0):
        return jax.random.uniform(self._next(), shape, jnp.bfloat16, lo, hi)
    def permutation(self, n):
        return jax.random.permutation(self._next(), n)


kernel_name = 'standalone__gqa_softmax__near_ridge'

def setup_inputs():
    _rng = _Rng(jax.random.key(int.from_bytes(__import__("os").urandom(4), "little")))
    _w = (lambda a: (lambda t: t.astype(jnp.bfloat16) if jnp.issubdtype(t.dtype, jnp.floating) else t)(jnp.asarray(a)))
    B, Hq, Hkv, Sq, Sk, D = 8, 16, 8, 160, 2048, 256
    return {
        "q": _w((lambda *s: _rng.normal(s) * 0.05)(B, Hq, Sq, D)),
        "k": _w((lambda *s: _rng.normal(s) * 3.2)(B, Hkv, Sk, D)),
        "v": _w((lambda *s: _rng.normal(s) * 0.05)(B, Hkv, Sk, D)),
    }

def reference(q, k, v):
    B, Hq, Sq, D = q.shape
    Hkv = k.shape[1]
    rep = Hq // Hkv
    k = jnp.repeat(k, rep, axis=1)
    v = jnp.repeat(v, rep, axis=1)
    scale = D ** -0.5
    scores = jnp.einsum("bhqd,bhkd->bhqk", q, k) * scale
    p = _softmax(scores, axis=-1)
    return jnp.einsum("bhqk,bhkd->bhqd", p, v)
```

```python
import math

import jax
import jax.numpy as jnp
from jax import lax
import jax.experimental.pallas as pl
import jax.experimental.pallas.tpu as pltpu

UN = 9
NB = 3
R = 3
RO = 9
NQ = 8
NP = 16
NC = 2
LEAD = 0.5

FLAGS = {"XLA_TPU_RESCHEDULE_DMA_DONES": True, "XLA_TPU_FORCE_LP_LLO_SCHEDULER": True}


@jax.jit
def pallas_standalone__gqa_softmax__near_ridge_kernel(q, k, v):
    B, Hq, Sq, D = q.shape
    _, Hkv, Sk, _ = k.shape
    M = (Hq // Hkv) * Sq
    N = B * Hkv
    UQ, UP, C = Sk // NQ, Sk // NP, Sk // NC
    assert UN % NB == 0 and UN % R == 0 and UN % RO == 0
    assert UQ % 128 == 0 and UP % 128 == 0 and D % 128 == 0 and M % 16 == 0
    rem = (N - 1) % UN
    base = 1 + rem
    assert N - base >= UN and N > NB
    c = (D ** -0.5) * math.log2(math.e)
    f32 = jnp.float32

    def body(q_hbm, k_hbm, v_hbm, o_hbm, q_buf, k_buf, v_buf, *rest):
        O, SO = rest[:RO], rest[RO:2 * RO]
        S, MX = rest[2 * RO:2 * RO + R], rest[2 * RO + R:2 * RO + 2 * R]
        l_ref, acc_ref, sem_q, sem_k, sem_v = rest[2 * RO + 2 * R:]

        def q_cp(i, sl):
            return pltpu.make_async_copy(q_hbm.at[i], q_buf.at[sl], sem_q.at[sl])

        def k_cp(i, sl, j):
            rows = pl.ds(j * C, C)
            return pltpu.make_async_copy(k_hbm.at[i, rows], k_buf.at[sl, rows], sem_k.at[sl, j])

        def v_cp(i, sl, j):
            rows = pl.ds(j * C, C)
            return pltpu.make_async_copy(v_hbm.at[i, rows], v_buf.at[sl, rows], sem_v.at[sl, j])

        def o_cp(i, ph):
            return pltpu.make_async_copy(O[ph % RO], o_hbm.at[i], SO[ph % RO])

        def when(cond, fn):
            if isinstance(cond, bool):
                if cond:
                    fn()
            else:
                pl.when(cond)(fn)

        def qk_unit(i, ph, u):
            sl, upc = ph % NB, NQ // NC
            if u % upc == 0:
                if u == 0:
                    q_cp(i, sl).wait()
                k_cp(i, sl, u // upc).wait()
            s = lax.dot_general(q_buf[sl], k_buf[sl, pl.ds(u * UQ, UQ), :],
                                (((1,), (1,)), ((), ())), preferred_element_type=f32) * c
            mx = s[:, 0:128]
            for j in range(1, UQ // 128):
                mx = jnp.maximum(mx, s[:, j * 128:(j + 1) * 128])
            if u > 0:
                mx = jnp.maximum(mx, MX[ph % R][...])
            if u == NQ - 1:
                mx = jnp.broadcast_to(jnp.max(mx, axis=-1, keepdims=True), (M, 128))
            MX[ph % R][...] = mx
            S[ph % R][:, pl.ds(u * UQ, UQ)] = s
            if u % upc == upc - 1:
                def refill():
                    k_cp(i + NB, sl, u // upc).start()
                    if u == NQ - 1:
                        q_cp(i + NB, sl).start()
                when(i + NB < N, refill)
                if isinstance(i, int) and i == 0:
                    v_cp(NB - 1, NB - 1, u // upc).start()

        def pv_unit(i, ph, u):
            sl, upc = ph % NB, NP // NC
            if u % upc == 0:
                v_cp(i, sl, u // upc).wait()
            mx = MX[ph % R][...]
            mx = jnp.concatenate([mx] * (UP // 128), axis=1)
            p = jnp.exp2(S[ph % R][:, pl.ds(u * UP, UP)] - mx)
            lsum = p[:, 0:128]
            for j in range(1, UP // 128):
                lsum = lsum + p[:, j * 128:(j + 1) * 128]
            if u == 0:
                l_ref[...] = lsum
            elif u < NP - 1:
                l_ref[...] += lsum
            else:
                lsum = l_ref[...] + lsum
            part = jnp.dot(p.astype(v_buf.dtype), v_buf[sl, pl.ds(u * UP, UP), :], preferred_element_type=f32)
            if u == 0:
                acc_ref[...] = part
            elif u < NP - 1:
                acc_ref[...] += part
            else:
                l = jnp.sum(lsum, axis=-1, keepdims=True)
                r = pl.reciprocal(l, approx=True)
                r = r * (2.0 - l * r)
                O[ph % RO][...] = ((acc_ref[...] + part) * r).astype(q.dtype)
            if u % upc == upc - 1:
                when(i + NB < N, lambda: v_cp(i + NB, sl, u // upc).start())

        def slot(t, ph, do_qk=True, do_pv=True):
            items = [(0.5, 2, "o_start", 0), (6.4, 2, "o_wait", 0)]
            if do_qk:
                items += [(u * 8 / NQ, 0, "qk", u) for u in range(NQ)]
            if do_pv:
                items += [(u * 8 / NP + LEAD, 1, "pv", u) for u in range(NP)]
            for _, _, kind, u in sorted(items):
                if kind == "qk":
                    qk_unit(t, ph, u)
                elif kind == "pv":
                    pv_unit(t - 1, ph - 1, u)
                elif kind == "o_start":
                    when(t >= 2, lambda: o_cp(t - 2, ph - 2).start())
                else:
                    when(t - 1 - RO >= 0, lambda: o_cp(t - 1 - RO, ph - 1).wait())

        def prologue(n, carry):
            i, j = n // NC, n % NC
            pl.when(j == 0)(lambda: q_cp(i, i).start())
            k_cp(i, i, j).start()
            pl.when(i > 0)(lambda: v_cp(jnp.maximum(i - 1, 0), jnp.maximum(i - 1, 0), j).start())
            return carry

        lax.fori_loop(0, NB * NC, prologue, 0)
        slot(0, 0, True, False)
        for t in range(1, base):
            slot(t, t)

        def loop(j, carry):
            t0 = base + UN * j
            for i in range(UN):
                slot(t0 + i, base + i)
            return carry

        lax.fori_loop(0, (N - base) // UN, loop, 0)
        slot(N, N, False, True)
        o_cp(N - 1, N - 1).start()
        for h in range(max(0, N - RO), N):
            o_cp(h, h).wait()

    out = pl.pallas_call(
        body,
        in_specs=[pl.BlockSpec(memory_space=pl.ANY)] * 3,
        out_specs=pl.BlockSpec(memory_space=pl.ANY),
        out_shape=jax.ShapeDtypeStruct((N, M, D), q.dtype),
        scratch_shapes=[
            pltpu.VMEM((NB, M, D), q.dtype),
            pltpu.VMEM((NB, Sk, D), k.dtype),
            pltpu.VMEM((NB, Sk, D), v.dtype),
            *[pltpu.VMEM((M, D), q.dtype) for _ in range(RO)],
            *[pltpu.SemaphoreType.DMA(()) for _ in range(RO)],
            *[pltpu.VMEM((M, Sk), f32) for _ in range(R)],
            *[pltpu.VMEM((M, 128), f32) for _ in range(R)],
            pltpu.VMEM((M, 128), f32),
            pltpu.VMEM((M, D), f32),
            pltpu.SemaphoreType.DMA((NB,)),
            pltpu.SemaphoreType.DMA((NB, NC)),
            pltpu.SemaphoreType.DMA((NB, NC)),
        ],
        compiler_params=pltpu.CompilerParams(vmem_limit_bytes=100 * 1024 * 1024, flags=FLAGS),
    )(q.reshape(N, M, D), k.reshape(N, Sk, D), v.reshape(N, Sk, D))
    return out.reshape(B, Hq, Sq, D)
```
